```python
import os as _os
_os.environ.setdefault("JAX_PLATFORMS", "cpu")
import jax
import jax.numpy as jnp

def _softmax(x, axis=-1):
    return jax.nn.softmax(x, axis=axis)
def _gelu(x):
    return jax.nn.gelu(x, approximate=True)
def _silu(x):
    return jax.nn.silu(x)
def _sigmoid(x):
    return jax.nn.sigmoid(x)
def _layernorm(x, axis=-1, eps=1e-5):
    m = jnp.mean(x, axis=axis, keepdims=True)
    v = jnp.var(x, axis=axis, keepdims=True)
    return (x - m) / jnp.sqrt(v + eps)
def _scatter_add(tgt, idx, src, axis=0):
    return tgt.at[idx].add(src)
def _segment_sum(src, seg, n):
    return jax.ops.segment_sum(src, seg, n)
class _Rng:
    def __init__(self, key):
        self._k = key
    def _next(self):
        self._k, sub = jax.random.split(self._k)
        return sub
    def normal(self, shape):
        return jax.random.normal(self._next(), shape, dtype=jnp.bfloat16)
    def randint(self, lo, hi, shape):
        return jax.random.randint(self._next(), shape, lo, hi, dtype=jnp.int32)
    def uniform(self, shape, lo=0.0, hi=1.0):
        return jax.random.uniform(self._next(), shape, jnp.bfloat16, lo, hi)
    def permutation(self, n):
        return jax.random.permutation(self._next(), n)


kernel_name = 'recurrent_scan__spectral_gfnet__swiglu_ffn__prompt'

def setup_inputs():
    _rng = _Rng(jax.random.key(int.from_bytes(__import__("os").urandom(4), "little")))
    _w = (lambda a: (lambda t: t.astype(jnp.bfloat16) if jnp.issubdtype(t.dtype, jnp.floating) else t)(jnp.asarray(a)))
    def _A_setup():
        B, S, D = 1, 2048, 640
        Df = D // 2 + 1
        return {
            "x": _w((lambda *s: _rng.normal(s) * 0.05)(B, S, D)),
            "w_r": _w((lambda *s: _rng.normal(s) * 0.05)(S, Df) * 0.02),
            "w_i": _w((lambda *s: _rng.normal(s) * 0.05)(S, Df) * 0.02),
        }
    _A_in = _A_setup()

    def _B_setup():
        B, S, D, F = 1, 2048, 640, 1536
        return {
            "x": _w((lambda *s: _rng.normal(s) * 0.05)(B, S, D)),
            "w_gate": _w((lambda *s: _rng.normal(s) * 0.05)(D, F)),
            "w_up": _w((lambda *s: _rng.normal(s) * 0.05)(D, F)),
            "w_down": _w((lambda *s: _rng.normal(s) * 0.05)(F, D)),
        }
    _B_in = _B_setup()

    return {
        "A_x": _A_in["x"],
        "A_w_r": _A_in["w_r"],
        "A_w_i": _A_in["w_i"],
        "B_x": _B_in["x"],
        "B_w_gate": _B_in["w_gate"],
        "B_w_up": _B_in["w_up"],
        "B_w_down": _B_in["w_down"],
    }

def reference(A_x, A_w_r, A_w_i, B_x, B_w_gate, B_w_up, B_w_down):
    def _A_ref(x, w_r, w_i):
        B, S, D = x.shape
        X = (lambda x, axes=(-2,-1): jnp.fft.rfft2(x.astype(jnp.float32), axes=axes))(x, axes=(-2, -1))
        W = w_r + 1j * w_i
        X = X * W
        y = (lambda x, s, axes=(-2,-1): jnp.fft.irfft2(x, s=s, axes=axes).astype(jnp.bfloat16))(X, (S, D), axes=(-2, -1))
        return y

    def _B_ref(x, w_gate, w_up, w_down):
        g = _silu(x @ w_gate)
        u = x @ w_up
        return (g * u) @ w_down

    x = A_x
    xn = _layernorm(x, axis=-1)
    s = _A_ref(xn, A_w_r, A_w_i)
    g = _silu(_B_ref(xn, B_w_gate, B_w_up, B_w_down))
    return x + s * g
```

```python
import math

import jax
import jax.numpy as jnp
import numpy as np
from jax import lax
from jax.experimental import pallas as pl
from jax.experimental.pallas import tpu as pltpu

S, D, F = 2048, 640, 1536
DF = D // 2 + 1
L = 128
RS = S // L
RD = D // L
NC = 3 * L
FB = 256
F32, BF16 = jnp.float32, jnp.bfloat16


def _col_freqs():
    l = np.arange(L)
    lo = l < 64
    ka = np.where(lo, 1 + 5 * l, 4 + 5 * (l - 64))
    kb = np.where(lo, 2 + 5 * l, 3 + 5 * (l - 64))
    kc = np.where(l <= 64, 5 * l, 0)
    return ka, kb, kc, np.where(lo, 1.0, -1.0), (l <= 64).astype(np.float64)


def _constants():
    ka, kb, kc, sg, vc = _col_freqs()
    n2 = np.arange(L)[:, None]

    def cs(k):
        th = 2.0 * np.pi * ((n2 * k[None, :]) % D) / D
        return np.cos(th), np.sin(th)

    def fam(k):
        c, s = cs(k)
        return np.block([[c, -s], [sg * s, sg * c]])

    fa, fb = fam(ka), fam(kb)
    c, s = cs(kc)
    fc = np.concatenate([c * vc, -s * vc], axis=1)
    wc = np.where((kc == 0) | (kc == D // 2), 1.0, 2.0)
    fwd_d = np.concatenate([fa, fb, fc], axis=0)
    inv_d = np.concatenate(
        [2.0 * fa.T, 2.0 * fb.T, fc.T * np.concatenate([wc, wc])[:, None]],
        axis=1) / (S * D)
    k = np.arange(RS)[:, None, None] + RS * np.arange(L)[None, :, None]
    ph = 2.0 * np.pi * ((k * np.arange(L)[None, None, :]) % S) / S
    c, s = np.cos(ph), np.sin(ph)
    fwd_s = np.concatenate([np.concatenate([c, s], 2),
                            np.concatenate([-s, c], 2)], 1)
    inv_s = np.transpose(fwd_s, (0, 2, 1))
    idx = np.zeros((8, NC), np.int32)
    idx[:] = np.concatenate([ka, kb, kc])[None, :]
    bf = lambda a: np.ascontiguousarray(a).astype(np.float32).astype(BF16)
    return bf(fwd_d), bf(inv_d), bf(fwd_s), bf(inv_s), idx


_FWD_D, _INV_D, _FWD_S, _INV_S, _IDX = _constants()
_C1, _C2 = math.cos(2 * math.pi / 5), math.cos(4 * math.pi / 5)
_S1, _S2 = math.sin(2 * math.pi / 5), math.sin(4 * math.pi / 5)


def _fft4(v, sign):
    (ar, ai), (br, bi), (cr, ci), (dr, di) = v
    er, ei, fr, fi = ar + cr, ai + ci, ar - cr, ai - ci
    gr, gi, hr, hi = br + dr, bi + di, br - dr, bi - di
    p, m = (fr - hi, fi + hr), (fr + hi, fi - hr)
    if sign < 0:
        p, m = m, p
    return [(er + gr, ei + gi), p, (er - gr, ei - gi), m]


def _twiddle(z, e, sign):
    r, i = z
    if e == 0:
        return z
    if e == 4:
        return (-i, r) if sign > 0 else (i, -r)
    c, s = math.cos(2 * math.pi * e / 16), sign * math.sin(2 * math.pi * e / 16)
    if e == 2:
        return ((r - i) * c, (r + i) * c) if sign > 0 else ((r + i) * c, (i - r) * c)
    if e == 6:
        return ((r + i) * c, (i - r) * c) if sign > 0 else ((r - i) * c, (r + i) * c)
    return (r * c - i * s, r * s + i * c)


def _fft16(v, sign):
    cols = [_fft4([v[b], v[4 + b], v[8 + b], v[12 + b]], sign) for b in range(4)]
    out = [None] * 16
    for k in range(4):
        res = _fft4([_twiddle(cols[b][k], b * k, sign) for b in range(4)], sign)
        for j in range(4):
            out[k + 4 * j] = res[j]
    return out


def _silu(v):
    h = 0.5 * v
    return h + h * jnp.tanh(h)


def _dot(a, b):
    return jnp.dot(a, b, preferred_element_type=F32)


def _kernel(x_hbm, wr_hbm, wi_hbm, wg_hbm, wu_hbm, wd_hbm, fd_hbm, gd_hbm, fs_hbm,
            gs_hbm, idx_hbm, o_hbm,
            x_v, wr_v, wi_v, wg_v, wu_v, wd_v, fd_v, gd_v, fs_v, gs_v, idx_v,
            xn_v, g_v, z_v, pr_v, pi_v, o_v, sem, xsem, osem):
    nb = S // FB

    def x_copy(b):
        return pltpu.make_async_copy(x_hbm.at[pl.ds(b * FB, FB)],
                                     x_v.at[pl.ds(b * FB, FB)], xsem.at[b])

    def o_copy(b):
        r = pl.ds(pl.multiple_of(b * FB, FB), FB)
        return pltpu.make_async_copy(o_v.at[r], o_hbm.at[r], osem.at[b])

    pairs = [(fd_hbm, fd_v), (wg_hbm, wg_v), (wu_hbm, wu_v), (wd_hbm, wd_v),
             (idx_hbm, idx_v), (wr_hbm, wr_v), (wi_hbm, wi_v), (fs_hbm, fs_v),
             (gs_hbm, gs_v), (gd_hbm, gd_v)]
    cp = [pltpu.make_async_copy(s, d, sem.at[i]) for i, (s, d) in enumerate(pairs)]
    x_copy(0).start()
    x_copy(1).start()
    for c in cp[:4]:
        c.start()
    for b in range(2, nb):
        x_copy(b).start()
    for c in cp[4:]:
        c.start()

    def ffn(blk):
        rows = pl.ds(pl.multiple_of(blk * FB, FB), FB)
        xn = xn_v[rows, :]
        h = (_silu(_dot(xn, wg_v[...])) * _dot(xn, wu_v[...])).astype(BF16)
        g_v[rows, :] = _silu(_dot(h, wd_v[...])).astype(BF16)

    def norm_dft(blk):
        rows = pl.ds(pl.multiple_of(blk * FB, FB), FB)
        x = x_v[rows, :].astype(F32)
        xc = x - jnp.mean(x, axis=-1, keepdims=True)
        var = jnp.mean(xc * xc, axis=-1, keepdims=True)
        xb = (xc * lax.rsqrt(var + 1e-5)).astype(BF16)
        xn_v[rows, :] = xb
        xn = xb.astype(F32)
        x0, x1, x2, x3, x4 = [xn[:, j * L:(j + 1) * L] for j in range(RD)]
        t1, t2, t3, t4 = x1 + x4, x2 + x3, x1 - x4, x2 - x3
        u0 = x0 + t1 + t2
        a1 = x0 + _C1 * t1 + _C2 * t2
        a2 = x0 + _C2 * t1 + _C1 * t2
        b1 = -_S1 * t3 - _S2 * t4
        b2 = _S1 * t4 - _S2 * t3
        cat = lambda a, b: jnp.concatenate([a.astype(BF16), b.astype(BF16)], axis=1)
        res = [_dot(cat(a1, b1), fd_v[0:2 * L, :]),
               _dot(cat(a2, b2), fd_v[2 * L:4 * L, :]),
               _dot(u0.astype(BF16), fd_v[4 * L:5 * L, :])]
        for j in range(FB // L):
            for t in range(3):
                for p in range(2):
                    z_v[blk * (FB // L) + j, p * L:(p + 1) * L, t * L:(t + 1) * L] = (
                        res[t][j * L:(j + 1) * L, p * L:(p + 1) * L])

    def radix16(grp0, ngrp, sign):
        for gi in range(ngrp):
            r = pl.multiple_of((grp0 + gi) * 8, 8)
            for t in range(3):
                cols = slice(t * L, (t + 1) * L)
                v = [(z_v[n, pl.ds(r, 8), cols], z_v[n, pl.ds(L + r, 8), cols])
                     for n in range(RS)]
                for n, (re, im) in enumerate(_fft16(v, sign)):
                    z_v[n, pl.ds(r, 8), cols] = re
                    z_v[n, pl.ds(L + r, 8), cols] = im

    def permute_w(row0, nrow):
        idx = idx_v[...]
        for src, dst in ((wr_v, pr_v), (wi_v, pi_v)):
            for c in range(nrow // 16):
                r = pl.multiple_of(row0 + c * 16, 16)
                tiles = [src[pl.ds(r, 16), 0:L], src[pl.ds(r, 16), L:2 * L],
                         jnp.concatenate([src[pl.ds(r, 16), 2 * L:DF],
                                          jnp.zeros((16, NC - DF), BF16)], axis=1)]
                tiles = [pltpu.bitcast(w, jnp.int32) for w in tiles]
                for t in range(3):
                    k = idx[:, t * L:(t + 1) * L]
                    g0, g1, g2 = [jnp.take_along_axis(w, k & (L - 1), axis=1)
                                  for w in tiles]
                    dst[t, pl.ds(pl.multiple_of(r // 2, 8), 8), :] = (
                        jnp.where(k < L, g0, jnp.where(k < 2 * L, g1, g2)))

    def spectral(m):
        wr, wi = [jnp.concatenate([p[t, pl.ds(m, L, stride=RS // 2), :]
                                   for t in range(3)], axis=1) for p in (pr_v, pi_v)]
        for j in range(2):
            k1 = 2 * m + j
            part = (lambda w: w << 16) if j == 0 else (lambda w: w & (-65536))
            cr = pltpu.bitcast(part(wr), F32)
            ci = pltpu.bitcast(part(wi), F32)
            xf = _dot(fs_v[k1], z_v[k1].astype(BF16))
            xr, xi = xf[:L], xf[L:]
            y = jnp.concatenate([(xr * cr - xi * ci).astype(BF16),
                                 (xr * ci + xi * cr).astype(BF16)], axis=0)
            z_v[k1] = _dot(gs_v[k1], y)

    def finish(blk):
        rows = pl.ds(pl.multiple_of(blk * FB, FB), FB)

        def spec(t):
            return jnp.concatenate(
                [jnp.concatenate(
                    [z_v[blk * (FB // L) + j, p * L:(p + 1) * L,
                         t * L:(t + 1) * L].astype(BF16) for p in range(2)], axis=1)
                 for j in range(FB // L)], axis=0)

        v1 = _dot(spec(0), gd_v[:, 0:2 * L])
        v2 = _dot(spec(1), gd_v[:, 2 * L:4 * L])
        u0 = _dot(spec(2), gd_v[:, 4 * L:5 * L])
        p1, q1, p2, q2 = v1[:, :L], v1[:, L:], v2[:, :L], v2[:, L:]
        e1 = u0 + _C1 * p1 + _C2 * p2
        e2 = u0 + _C2 * p1 + _C1 * p2
        o1 = _S1 * q1 + _S2 * q2
        o2 = _S2 * q1 - _S1 * q2
        ys = [u0 + p1 + p2, e1 - o1, e2 - o2, e2 + o2, e1 + o1]
        for j in range(RD):
            cols = slice(j * L, (j + 1) * L)
            o_v[rows, cols] = (x_v[rows, cols].astype(F32)
                               + ys[j] * g_v[rows, cols].astype(F32)).astype(BF16)

    def loop(n, body):
        lax.fori_loop(0, n, lambda i, c: (body(i), c)[1], 0)

    for c in cp[:4]:
        c.wait()

    def phase_a(i):
        x_copy(2 * i).wait()
        x_copy(2 * i + 1).wait()
        norm_dft(2 * i)
        norm_dft(2 * i + 1)
        ffn(i)
    loop(4, phase_a)

    for c in cp[4:7]:
        c.wait()

    def phase_b1(i):
        radix16(i * 8, 8, -1)
        permute_w(i * (S // 2), S // 2)
        ffn(4 + i)
    loop(2, phase_b1)

    cp[7].wait()
    cp[8].wait()
    loop(RS // 2, spectral)

    def phase_b3(i):
        radix16(i * 8, 8, 1)
        ffn(6 + i)
    loop(2, phase_b3)

    cp[9].wait()

    def phase_c(i):
        finish(i)
        o_copy(i).start()
    loop(nb, phase_c)
    for b in range(nb):
        o_copy(b).wait()


@jax.jit
def pallas_recurrent_scan__spectral_gfnet__swiglu_ffn__prompt_kernel(
    A_x: jax.Array,
    A_w_r: jax.Array,
    A_w_i: jax.Array,
    B_x: jax.Array,
    B_w_gate: jax.Array,
    B_w_up: jax.Array,
    B_w_down: jax.Array,
):
    del B_x
    vm = pltpu.VMEM
    out = pl.pallas_call(
        _kernel,
        out_shape=jax.ShapeDtypeStruct((S, D), BF16),
        in_specs=[pl.BlockSpec(memory_space=pl.ANY)] * 11,
        out_specs=pl.BlockSpec(memory_space=pl.ANY),
        scratch_shapes=[
            vm((S, D), BF16), vm((S, DF), BF16), vm((S, DF), BF16),
            vm((D, F), BF16), vm((D, F), BF16), vm((F, D), BF16),
            vm(_FWD_D.shape, BF16), vm(_INV_D.shape, BF16),
            vm(_FWD_S.shape, BF16), vm(_INV_S.shape, BF16), vm(_IDX.shape, jnp.int32),
            vm((S, D), BF16), vm((S, D), BF16), vm((RS, 2 * L, NC), F32),
            vm((3, S // 2, L), jnp.int32), vm((3, S // 2, L), jnp.int32),
            vm((S, D), BF16),
            pltpu.SemaphoreType.DMA((10,)), pltpu.SemaphoreType.DMA((S // FB,)),
            pltpu.SemaphoreType.DMA((S // FB,)),
        ],
        compiler_params=pltpu.CompilerParams(vmem_limit_bytes=100 * 1024 * 1024),
    )(A_x.reshape(S, D), A_w_r, A_w_i, B_w_gate, B_w_up, B_w_down,
      _FWD_D, _INV_D, _FWD_S, _INV_S, _IDX)
    return out.reshape(A_x.shape)
```

```python
import functools
import math

import jax
import jax.numpy as jnp
import numpy as np
from jax import lax
from jax.experimental import pallas as pl
from jax.experimental.pallas import tpu as pltpu

S, D, F = 2048, 640, 1536
DF = D // 2 + 1
L = 128
LS = 64
RS = S // LS
NT = S // L
RD = D // L
NC = 3 * L
FB = 256
PS = RS + 1
HM = FB // 2
NP = F // (2 * L)
NA = 4
HB = 64
F32, BF16, U32 = jnp.float32, jnp.bfloat16, jnp.uint32
HI16 = np.uint32(0xFFFF0000)


_RUNS = ((1, 6, 4, 9), (2, 7, 3, 8), (0, 5))


def _constants():
    i = np.arange(32)
    ka, kb, k0 = [np.concatenate([c + 10 * i for c in run]) for run in _RUNS]
    sg = np.where(np.arange(L) < 64, 1.0, -1.0)
    n2 = np.arange(L)[:, None]

    def cs(k):
        th = 2.0 * np.pi * ((n2 * k[None, :]) % D) / D
        return np.cos(th), np.sin(th)

    fwd_d, inv_d = [], []
    for k in (ka, kb):
        c, s = cs(k)
        fwd_d += [c, sg * s - c, -sg * s - c]
        inv_d += [2.0 * c.T, -2.0 * (sg * s + c).T, 2.0 * (sg * s - c).T]
    c, s = cs(np.concatenate([k0, [D // 2]]))
    packed = np.concatenate([c, -s[:, 1:64]], axis=1)
    twice = np.full(L, 2.0)
    twice[[0, 64]] = 1.0
    fwd_d = np.concatenate(fwd_d + [packed], axis=0)
    inv_d = np.concatenate(inv_d + [(packed * twice).T], axis=0) / (S * D)
    k = np.arange(RS)[:, None, None] + RS * np.arange(LS)[None, :, None]
    ph = 2.0 * np.pi * ((k * np.arange(LS)[None, None, :]) % S) / S
    c, s = np.cos(ph), np.sin(ph)
    fwd_s = np.concatenate([np.concatenate([c, s], 2),
                            np.concatenate([-s, c], 2)], 1)
    inv_s = np.transpose(fwd_s, (0, 2, 1))

    def words(a):
        h = np.ascontiguousarray(a).astype(np.float32).astype(BF16).view(np.uint16)
        h = h.astype(np.uint32)
        return h[..., 0::2, :] | (h[..., 1::2, :] << 16)

    return words(fwd_d), words(inv_d), words(fwd_s), words(inv_s)


_FWD_D, _INV_D, _FWD_S, _INV_S = _constants()
_C1, _C2 = math.cos(2 * math.pi / 5), math.cos(4 * math.pi / 5)
_S1, _S2 = math.sin(2 * math.pi / 5), math.sin(4 * math.pi / 5)


def _fft4(v, sign):
    (ar, ai), (br, bi), (cr, ci), (dr, di) = v
    er, ei, fr, fi = ar + cr, ai + ci, ar - cr, ai - ci
    gr, gi, hr, hi = br + dr, bi + di, br - dr, bi - di
    p, m = (fr - hi, fi + hr), (fr + hi, fi - hr)
    if sign < 0:
        p, m = m, p
    return [(er + gr, ei + gi), p, (er - gr, ei - gi), m]


def _twiddle(z, e, n, sign):
    r, i = z
    if 2 * e >= n:
        r, i = _twiddle(z, e - n // 2, n, sign)
        return -r, -i
    if e == 0:
        return z
    if 4 * e == n:
        return (-i, r) if sign > 0 else (i, -r)
    c, s = math.cos(2 * math.pi * e / n), sign * math.sin(2 * math.pi * e / n)
    if 8 * e == n:
        return ((r - i) * c, (r + i) * c) if sign > 0 else ((r + i) * c, (i - r) * c)
    if 8 * e == 3 * n:
        return ((r + i) * c, (i - r) * c) if sign > 0 else ((r - i) * c, (r + i) * c)
    return (r * c - i * s, r * s + i * c)


def _fft(v, sign):
    n = len(v)
    if n == 2:
        (ar, ai), (br, bi) = v
        return [(ar + br, ai + bi), (ar - br, ai - bi)]
    if n == 4:
        return _fft4(v, sign)
    m = n // 4
    cols = [_fft4([v[m * a + b] for a in range(4)], sign) for b in range(m)]
    out = [None] * n
    for k in range(4):
        res = _fft([_twiddle(cols[b][k], b * k, n, sign) for b in range(m)], sign)
        for j in range(m):
            out[k + 4 * j] = res[j]
    return out


def _silu(v):
    h = 0.5 * v
    return h + h * jnp.tanh(h)


def _dot(a, b):
    return jnp.dot(a, b, preferred_element_type=F32)


def _kernel(x_hbm, wr_hbm, wi_hbm, wg_hbm, wu_hbm, wd_hbm, fd_hbm, gd_hbm, fs_hbm,
            gs_hbm, zero_hbm, o_hbm,
            x_v, wr_v, wi_v, wg_v, wu_v, wd_v, fd_v, gd_v, fs_v, gs_v, zero_v,
            xn_v, su_v, sx_v, sd_v, sr_v, h_v, g_v, z_v, ws_v, p_v, o_v, sem, fsem, wsem, xsem, osem):
    nb = S // FB
    lane = lax.broadcasted_iota(jnp.int32, (1, L), 1)
    sigma = jnp.where(lane < 64, 1.0, -1.0).astype(F32)
    table = lambda ref, j: bf(ref[j * L // 2:(j + 1) * L // 2, :])
    bf = lambda w: pltpu.bitcast(w, BF16)
    wd32 = lambda v: pltpu.bitcast(v, U32)
    wrows = lambda r0, n: pl.ds(pl.multiple_of(r0 // 2, n // 2), n // 2)
    P = functools.partial

    def x_copy(b):
        return pltpu.make_async_copy(x_hbm.at[pl.ds(b * FB, FB)],
                                     x_v.at[pl.ds(b * FB, FB)], xsem.at[b])

    def o_copy(b):
        r = pl.ds(b * FB, FB)
        return pltpu.make_async_copy(o_v.at[r], o_hbm.at[r], osem.at[b])

    def start(cs):
        for c in cs:
            c.start()

    def wait(cs):
        for c in cs:
            c.wait()

    edges = (0, 128, 384, 896, F)
    fcp = [[pltpu.make_async_copy(src.at[:, pl.ds(lo, hi - lo)], dst.at[:, pl.ds(lo, hi - lo)],
                                  fsem.at[2 * c + j])
            for j, (src, dst) in enumerate(((wg_hbm, wg_v), (wu_hbm, wu_v)))]
           for c, (lo, hi) in enumerate(zip(edges[:-1], edges[1:]))]
    fcp.append([pltpu.make_async_copy(wd_hbm, wd_v, fsem.at[10])])
    pairs = [(fd_hbm, fd_v), (fs_hbm, fs_v), (gs_hbm, gs_v)] + [
        (gd_hbm.at[h], gd_v.at[h]) for h in (pl.ds(0, 2 * L), pl.ds(2 * L, 3 * L // 2))]
    cp = [pltpu.make_async_copy(s, d, sem.at[i]) for i, (s, d) in enumerate(pairs)]
    wcp = [pltpu.make_async_copy(src, dst, wsem.at[j])
           for j, (src, dst) in enumerate(((wr_hbm, wr_v), (wi_hbm, wi_v)))]

    dep = []

    def tie(w):
        if not dep:
            return w
        return w | jnp.tile(dep[0], (w.shape[0] // 8, w.shape[1] // L))

    def spreader(fill, total):
        state = [0, 0]

        def step(tiles):
            state[0] += tiles
            upto = (len(fill) * state[0] + total - 1) // total
            for f in fill[state[1]:upto]:
                f()
            state[1] = max(state[1], upto)
        return step

    def lhs_terms(a11, a12, a21, a22):
        return [v.astype(BF16) for v in
                (a11 + a22, a21 + a22, a11, a22, a11 + a12, a21 - a11, a12 - a22)]

    def rhs_terms(*b):
        b = [pltpu.bitcast(v, U32) for v in b]
        b = [bf(v) for v in (tie(b[0]), b[1], b[2], tie(b[3]))]
        b11, b12, b21, b22 = [v.astype(F32) for v in b]
        return [v.astype(BF16) for v in
                (b11 + b22, b[0], b12 - b22, b21 - b11, b[3], b11 + b12, b21 + b22)]

    def combine(m):
        return (m[0] + m[3] - m[4] + m[6], m[2] + m[4], m[1] + m[3], m[0] - m[1] + m[2] + m[5])

    def tile(j, n=1):
        return slice(j * L, (j + n) * L)

    def wtile(j):
        return slice(j * L // 2, (j + 1) * L // 2)

    def prep_up(p, w, k):
        src = (wg_v, wu_v)[w]
        terms = rhs_terms(*[src[tile(r + k), tile(2 * p + c)] for r in (0, 2) for c in (0, 1)])
        for q, v in enumerate(terms):
            su_v[w, q, wtile(k), tile(p)] = wd32(v)
        sx_v[w, :, tile(2 * p + k)] = wd32(src[tile(4), tile(2 * p + k)])

    def prep_down(p, j):
        if j == 2:
            b1, b2 = [wd32(wd_v[tile(2 * p + r), tile(4)]) for r in (0, 1)]
            sr_v[0, wtile(p), :] = wd32((bf(b1).astype(F32) - bf(b2).astype(F32)).astype(BF16))
            sr_v[1, wtile(p), :] = b1
            sr_v[2, wtile(p), :] = b2
            return
        terms = rhs_terms(*[wd_v[tile(2 * p + r), tile(c + j)] for r in (0, 1) for c in (0, 2)])
        for q, v in enumerate(terms):
            sd_v[q, wtile(p), tile(j)] = wd32(v)

    def up_tiles(blk, pairs, put, qs, rest_first):
        halves = [wrows(blk * FB + i * HM, HM) for i in (0, 1)]
        terms, acc, tiles = [], {}, []

        def lhs(q, k):
            if not terms:
                terms.extend(lhs_terms(*[bf(xn_v[r, tile(c, 2)]).astype(F32)
                                         for r in halves for c in (0, 2)]))
            return terms[q][:, tile(k)]

        def done(p):
            gate, up = [[c + acc.pop((w, p, 7 + i)) for i, c in
                         enumerate(combine([acc.pop((w, p, q)) for q in range(7)]))]
                        for w in (0, 1)]
            put(p, lhs_terms(*[_silu(g) * u for g, u in zip(gate, up)]))

        for p in pairs:
            for w in (0, 1):
                main = [((w, p, q), P(lhs, q, k),
                           P(lambda w, q, k, p: bf(su_v[w, q, wtile(k), tile(p)]), w, q, k, p),
                           None)
                          for q in qs for k in (0, 1)]
                rest = [((w, p, 7 + 2 * i + c), P(lambda i: bf(xn_v[halves[i], tile(4)]), i),
                           P(lambda w, j: bf(sx_v[w, :, tile(j)]), w, 2 * p + c), None)
                          for i in (0, 1) for c in (0, 1)]
                tiles += rest + main if rest_first else main + rest
            tiles[-1] = tiles[-1][:3] + (P(done, p),)
        return [(acc,) + t for t in tiles]

    def down_tiles(blk, get, qs):
        halves = [pl.ds(pl.multiple_of(blk * FB + i * HM, HM), HM) for i in (0, 1)]
        acc, tiles = {}, []

        def done(c):
            for i, v in enumerate(combine([acc.pop((c, q)) for q in range(7)])):
                g_v[halves[i // 2], tile(2 * (i % 2) + c)] = _silu(v)

        def done_last():
            g_v[halves[0], tile(4)] = _silu(acc.pop(0) + acc.pop(1))
            g_v[halves[1], tile(4)] = _silu(acc.pop(2) - acc.pop(3))

        order = [(q, p) for q in qs for p in range(NP)]
        late = [(q, NP - 1) for q in qs[:3]]
        first = [t for t in order[:3 * NP] if t not in late] + late + order[3 * NP:]
        for c, terms in enumerate((first, order)):
            tiles += [((c, q), P(get, q, p),
                       P(lambda q, p, c: bf(sd_v[q, wtile(p), tile(c)]), q, p, c), None)
                      for q, p in terms]
            tiles[-1] = tiles[-1][:3] + (P(done, c),)
        tiles += [(i, P(get, q, p), P(lambda j, p: bf(sr_v[j, wtile(p), :]), j, p), None)
                  for i, (q, j) in enumerate(((2, 0), (4, 2), (1, 1), (3, 0))) for p in range(NP)]
        tiles[-1] = tiles[-1][:3] + (done_last,)
        return [(acc,) + t for t in tiles]

    def run(tiles, fill, pinned=0, rnd=4):
        step = spreader(fill, len(tiles))
        hist, pend = [], []

        def retire(acc, key, then, r):
            if pinned:
                hist.append(pltpu.bitcast(r[-8:], U32) & (hist or [zero_v[...]])[-1])
                dep[:] = hist[-pinned:][:1] if len(hist) >= pinned else []
            acc[key] = acc[key] + r if key in acc else r
            if then:
                then()

        for i in range(0, len(tiles), rnd):
            new = [(acc, key, then, _dot(lhs(), rhs()))
                   for acc, key, lhs, rhs, then in tiles[i:i + rnd]]
            for t in pend:
                retire(*t)
            step(len(new))
            pend = new
        for t in pend:
            retire(*t)
        dep[:] = []

    def ffn(blk, fill, lag, rnd, qs, rest_first=False, extra=None):
        hs = {}
        tiles = up_tiles(blk, range(NP), hs.__setitem__, qs, rest_first)
        if extra is not None:
            tiles += down_tiles(extra, lambda q, p: bf(h_v[extra, q, :, tile(p)]), qs)
        run(tiles + down_tiles(blk, lambda q, p: hs[p][q], qs), fill, lag, rnd)

    def norm(hb):
        rows = pl.ds(pl.multiple_of(hb * HB, HB), HB)
        x = bf(tie(pltpu.bitcast(x_v[rows, :], U32))).astype(F32)
        xc = x - jnp.mean(x, axis=-1, keepdims=True)
        var = jnp.mean(xc * xc, axis=-1, keepdims=True)
        xn_v[wrows(hb * HB, HB), :] = wd32((xc * lax.rsqrt(var + 1e-5)).astype(BF16))

    def dft_d(blk):
        lhs = []

        def radix5():
            xn = bf(tie(xn_v[wrows(blk * FB, FB), :])).astype(F32)
            x0, x1, x2, x3, x4 = [xn[:, j * L:(j + 1) * L] for j in range(RD)]
            t1, t2, t3, t4 = x1 + x4, x2 + x3, x1 - x4, x2 - x3
            lhs.append((x0 + _C1 * t1 + _C2 * t2, -_S1 * t3 - _S2 * t4))
            lhs.append((x0 + _C2 * t1 + _C1 * t2, _S1 * t4 - _S2 * t3))
            lhs[:] = [[v.astype(BF16) for v in (a + b, b, a)] for a, b in lhs]
            lhs.append((x0 + t1 + t2).astype(BF16))

        def mm(t):
            if t < 2:
                m = [_dot(v, table(fd_v, 3 * t + j)) for j, v in enumerate(lhs[t])]
                res = (m[0] + m[1], (m[0] + m[2]) * sigma)
            else:
                m = _dot(lhs[t], table(fd_v, 6))
                res = (jnp.where(lane <= 64, m, 0.0),
                       jnp.where((lane >= 1) & (lane < 64), pltpu.roll(m, 64, 1), 0.0))
            for j in range(FB // LS):
                for p in range(2):
                    z_v[blk * (FB // LS) + j, p * LS:(p + 1) * LS, t * L:(t + 1) * L] = (
                        res[p][j * LS:(j + 1) * LS])

        return [radix5] + [P(mm, t) for t in range(3)]

    def norms(blk):
        return [P(norm, blk * (FB // HB) + j) for j in range(FB // HB)]

    def butterflies(r, t, sign):
        cols = slice(t * L, (t + 1) * L)
        mid = {}
        held = lambda z: (pltpu.bitcast(tie(pltpu.bitcast(z[0], U32)), F32), z[1])

        def first(b):
            v = [(z_v[n, pl.ds(r, 8), cols], z_v[n, pl.ds(LS + r, 8), cols])
                 for n in range(b, RS, 8)]
            v[0] = held(v[0])
            for k, w in enumerate(_fft4(v, sign)):
                mid[b, k] = _twiddle(w, b * k, RS, sign)

        def second(k):
            res = _fft([held(mid[0, k])] + [mid[b, k] for b in range(1, 8)], sign)
            for j, (re, im) in enumerate(res):
                z_v[k + 4 * j, pl.ds(r, 8), cols] = re
                z_v[k + 4 * j, pl.ds(LS + r, 8), cols] = im

        return [P(first, b) for b in range(8)] + [P(second, k) for k in range(4)]

    def permute_w(st):
        lanes = tile(st)

        def stage():
            for j, src in enumerate((wr_v, wi_v)):
                ws_v[2 * st + j, 0:D // 4, :] = wd32(src[0:D // 2, lanes])

        def word(c):
            r, i = [ws_v[2 * st + j, pl.ds(c // 2, 32, stride=5), :] for j in (0, 1)]
            return (r & HI16) | (i >> 16) if c % 2 else (r << 16) | (i & 0xFFFF)

        def turn(t):
            rows = [word(c) for c in _RUNS[t]]
            if t == 2:
                nr, ni = [pltpu.bitcast(n[D // 2:DF, lanes].astype(F32), U32)
                          for n in (wr_v, wi_v)]
                rows.append(jnp.broadcast_to((nr & HI16) | (ni >> 16), (64, L)))
            w = jnp.concatenate(rows, axis=0).T
            for j in range(L // RS):
                p_v[t, pl.ds((st * (L // RS) + j) * PS, RS), :] = w[j * RS:(j + 1) * RS]

        return [stage] + [P(turn, t) for t in range(3)]

    def spectral(k1):
        y = []

        def forward():
            xf = _dot(bf(fs_v[k1]), z_v[k1].astype(BF16))
            y.append(xf)

        def apply():
            w = jnp.concatenate([p_v[t, pl.ds(k1, LS, stride=PS), :]
                                 for t in range(3)], axis=1)
            cr = pltpu.bitcast(w & HI16, F32)
            ci = pltpu.bitcast(w << 16, F32)
            xr, xi = y[0][:LS], y[0][LS:]
            y.append(jnp.concatenate([(xr * cr - xi * ci).astype(BF16),
                                      (xr * ci + xi * cr).astype(BF16)], axis=0))

        def inverse():
            z_v[k1] = _dot(bf(gs_v[k1]), y[1])

        return [forward, apply, inverse]

    def finish(blk):
        rows = pl.ds(pl.multiple_of(blk * FB, FB), FB)

        v = []

        def mm(t):
            re, im = [jnp.concatenate(
                [z_v[blk * (FB // LS) + j, p * LS:(p + 1) * LS, t * L:(t + 1) * L]
                 for j in range(FB // LS)], axis=0) for p in range(2)]
            if t < 2:
                im = im * sigma
                m = [_dot(u.astype(BF16), table(gd_v, 3 * t + j))
                     for j, u in enumerate((re + im, im, re))]
                v.extend([m[0] + m[1], m[0] + m[2]])
            else:
                u = jnp.where(lane <= 64, re, pltpu.roll(im, 64, 1))
                v.append(_dot(u.astype(BF16), table(gd_v, 6)))

        def put(j, y):
            cols = slice(j * L, (j + 1) * L)
            o_v[rows, cols] = (x_v[rows, cols].astype(F32) + y * g_v[rows, cols]).astype(BF16)

        def outer():
            p1, q1, p2, q2, u0 = v
            e, o = u0 + _C1 * p1 + _C2 * p2, _S1 * q1 + _S2 * q2
            put(1, e - o)
            put(4, e + o)

        def inner():
            p1, q1, p2, q2, u0 = v
            e, o = u0 + _C2 * p1 + _C1 * p2, _S2 * q1 - _S1 * q2
            put(2, e - o)
            put(3, e + o)
            put(0, u0 + p1 + p2)
            o_copy(blk).start()

        return [P(mm, t) for t in range(3)] + [outer, inner]

    def mix(*lists):
        keyed = [((i + 0.5) / len(l), k, f) for k, l in enumerate(lists) for i, f in enumerate(l)]
        return [f for _, _, f in sorted(keyed, key=lambda e: e[:2])]

    def bfly(sign):
        return [f for r in range(0, LS, 8) for t in range(3) for f in butterflies(r, t, sign)]

    idle = [lambda: None]
    xs = [x_copy(b) for b in range(nb)]
    zcp = [pltpu.make_async_copy(zero_hbm, zero_v, wsem.at[2])]
    start(fcp[0] + xs[:2] + zcp)
    wait(fcp[0][:1])
    start(fcp[1])
    wait(fcp[0][1:] + xs[:2] + zcp)
    for f in norms(0):
        f()
    later = (fcp[2], fcp[3] + xs[2:3], fcp[4] + cp[:1], xs[3:])

    hs, acc = {}, {}

    def settle(b, j):
        hs[b, j] = _silu(acc.pop((0, b, j))) * acc.pop((1, b, j))
        if j % 2:
            even, odd = hs.pop((b, j - 1)), hs.pop((b, j))
            for q, v in enumerate(lhs_terms(even[:HM], odd[:HM], even[HM:], odd[HM:])):
                h_v[b, q, :, tile(j // 2)] = wd32(v)

    for c, (lo, hi) in enumerate(zip(edges[:-1], edges[1:])):
        wait((fcp[c] if c else []) + (xs[2:3] if c == 3 else []))
        start(later[c])
        fill = [P(prep_up, p, w, k) for p in range(lo // (2 * L), hi // (2 * L))
                for w in (0, 1) for k in (0, 1)]
        more = {0: norms(1) + idle * 8, 3: norms(2)}.get(c, [])
        run([(acc, (w, b, j), P(lambda b, k: bf(xn_v[wrows(b * FB, FB), tile(k)]), b, k),
              P(lambda src, k, j: src[tile(k), tile(j)], src, k, j),
              P(settle, b, j) if (w, k) == (1, RD - 1) else None)
             for j in range(lo // L, hi // L) for b in (0, 1)
             for w, src in enumerate((wg_v, wu_v)) for k in range(RD)],
            (mix(fill, more) if fill and more else fill + more)
            + idle * (1, 1, 2, 0)[c],
            *((6, 1), (10, 4), (0, 4), (10, 4))[c])

    wait(fcp[4] + cp[:1] + xs[3:6])
    start(wcp + cp[1:])

    work = [f for b in range(4) for f in (norms(3 + b) if b < 3 else []) + dft_d(b)]
    prep = [P(prep_down, p, j) for p in range(NP) for j in range(3)]
    ffn(2, mix(work, prep + idle * 24) + idle * 2, 12, 3, (2, 4, 1, 3, 0, 6, 5))
    wait(xs[6:] + wcp)
    work = [f for b in range(4, nb) for f in (norms(2 + b) if b < 6 else []) + dft_d(b)]
    ffn(3, mix(work, [f for st in range(NA) for f in permute_w(st)]) + idle * 2,
        2, 1, (2, 4, 1, 3, 0, 6, 5), rest_first=True)

    wait(cp[1:2])
    ffn(4, mix(bfly(-1), [f for st in range(NA, NT) for f in permute_w(st)] + idle * 5),
        6, 2, range(7), rest_first=True, extra=0)

    wait(cp[2:3])
    sp = [spectral(k) for k in range(RS)]
    ffn(5, [sp[k - 2 * j][j] for k in range(RS + 4) for j in (2, 1, 0) if 0 <= k - 2 * j < RS],
        0, 1, (0, 5, 1, 3, 6, 4, 2))

    wait(cp[3:4])
    ffn(6, bfly(1), 6, 2, range(7), rest_first=True, extra=1)

    wait(cp[4:])
    fs = [finish(b) for b in range(nb)]
    ffn(7, fs[0][:3] + [f for b in range(nb - 1) for f in fs[b + 1][:3] + fs[b][3:]] + idle * 3,
        0, 1, (0, 5, 1, 3, 6, 4, 2))
    for f in fs[-1][3:]:
        f()
    wait([o_copy(b) for b in range(nb)])


@jax.jit
def pallas_recurrent_scan__spectral_gfnet__swiglu_ffn__prompt_kernel(
    A_x: jax.Array,
    A_w_r: jax.Array,
    A_w_i: jax.Array,
    B_x: jax.Array,
    B_w_gate: jax.Array,
    B_w_up: jax.Array,
    B_w_down: jax.Array,
):
    del B_x
    vm = pltpu.VMEM
    out = pl.pallas_call(
        _kernel,
        out_shape=jax.ShapeDtypeStruct((S, D), BF16),
        in_specs=[pl.BlockSpec(memory_space=pltpu.HBM)] * 11,
        out_specs=pl.BlockSpec(memory_space=pltpu.HBM),
        scratch_shapes=[
            vm((S, D), BF16), vm((DF, S), BF16), vm((DF, S), BF16),
            vm((D, F), BF16), vm((D, F), BF16), vm((F, D), BF16),
            vm(_FWD_D.shape, U32), vm(_INV_D.shape, U32),
            vm(_FWD_S.shape, U32), vm(_INV_S.shape, U32), vm((8, L), U32),
            vm((S // 2, D), U32), vm((2, 7, L, F // 2), U32), vm((2, L // 2, F), U32),
            vm((7, F // 4, 2 * L), U32), vm((3, F // 4, L), U32), vm((2, 7, HM // 2, F // 2), U32),
            vm((S, D), F32), vm((RS, 2 * LS, NC), F32),
            vm((2 * NT, D // 4 + 8, L), U32), vm((3, (LS + 8) * PS, L), U32),
            vm((S, D), BF16),
            pltpu.SemaphoreType.DMA((5,)), pltpu.SemaphoreType.DMA((11,)),
            pltpu.SemaphoreType.DMA((3,)), pltpu.SemaphoreType.DMA((S // FB,)),
            pltpu.SemaphoreType.DMA((S // FB,)),
        ],
        compiler_params=pltpu.CompilerParams(vmem_limit_bytes=100 * 1024 * 1024),
    )(A_x.reshape(S, D), A_w_r.T, A_w_i.T, B_w_gate, B_w_up, B_w_down,
      _FWD_D, _INV_D, _FWD_S, _INV_S, np.zeros((8, L), np.uint32))
    return out.reshape(A_x.shape)
```
